```python
import os as _os
_os.environ.setdefault("JAX_PLATFORMS", "cpu")
import jax
import jax.numpy as jnp

def _softmax(x, axis=-1):
    return jax.nn.softmax(x, axis=axis)
def _gelu(x):
    return jax.nn.gelu(x, approximate=True)
def _silu(x):
    return jax.nn.silu(x)
def _sigmoid(x):
    return jax.nn.sigmoid(x)
def _layernorm(x, axis=-1, eps=1e-5):
    m = jnp.mean(x, axis=axis, keepdims=True)
    v = jnp.var(x, axis=axis, keepdims=True)
    return (x - m) / jnp.sqrt(v + eps)
def _scatter_add(tgt, idx, src, axis=0):
    return tgt.at[idx].add(src)
def _segment_sum(src, seg, n):
    return jax.ops.segment_sum(src, seg, n)
class _Rng:
    def __init__(self, key):
        self._k = key
    def _next(self):
        self._k, sub = jax.random.split(self._k)
        return sub
    def normal(self, shape):
        return jax.random.normal(self._next(), shape, dtype=jnp.bfloat16)
    def randint(self, lo, hi, shape):
        return jax.random.randint(self._next(), shape, lo, hi, dtype=jnp.int32)
    def uniform(self, shape, lo=0.0, hi=1.0):
        return jax.random.uniform(self._next(), shape, jnp.bfloat16, lo, hi)
    def permutation(self, n):
        return jax.random.permutation(self._next(), n)


kernel_name = 'standalone__gqa_softmax__near_ridge'

def setup_inputs():
    _rng = _Rng(jax.random.key(int.from_bytes(__import__("os").urandom(4), "little")))
    _w = (lambda a: (lambda t: t.astype(jnp.bfloat16) if jnp.issubdtype(t.dtype, jnp.floating) else t)(jnp.asarray(a)))
    B, Hq, Hkv, Sq, Sk, D = 16, 32, 32, 368, 512, 192
    return {
        "q": _w((lambda *s: _rng.normal(s) * 0.4)(B, Hq, Sq, D)),
        "k": _w((lambda *s: _rng.normal(s) * 0.4)(B, Hkv, Sk, D)),
        "v": _w((lambda *s: _rng.normal(s) * 0.05)(B, Hkv, Sk, D)),
    }

def reference(q, k, v):
    B, Hq, Sq, D = q.shape
    Hkv = k.shape[1]
    rep = Hq // Hkv
    k = jnp.repeat(k, rep, axis=1)
    v = jnp.repeat(v, rep, axis=1)
    scale = D ** -0.5
    scores = jnp.einsum("bhqd,bhkd->bhqk", q, k) * scale
    p = _softmax(scores, axis=-1)
    return jnp.einsum("bhqk,bhkd->bhqd", p, v)
```

```python
import math

import jax
import jax.numpy as jnp
from jax import lax
import jax.experimental.pallas as pl
import jax.experimental.pallas.tpu as pltpu


@jax.jit
def pallas_standalone__gqa_softmax__near_ridge_kernel(q: jax.Array, k: jax.Array, v: jax.Array):
    B, Hq, Sq, D = q.shape
    _, Hkv, Sk, _ = k.shape
    assert Hq == Hkv
    N = B * Hq
    hb = 8
    c = (D ** -0.5) * math.log2(math.e)

    def kernel(q_ref, k_ref, v_ref, o_ref):
        for h in range(hb):
            sT = lax.dot_general(k_ref[h], q_ref[h], (((0,), (0,)), ((), ())),
                                 preferred_element_type=jnp.float32)
            m = jnp.max(sT, axis=0, keepdims=True)
            p = jnp.exp2((sT - m) * c)
            l = jnp.sum(p, axis=0, keepdims=True)
            oT = jnp.dot(v_ref[h], p.astype(jnp.bfloat16), preferred_element_type=jnp.float32)
            o_ref[h] = (oT * (1.0 / l)).astype(o_ref.dtype)

    qt = jnp.swapaxes(q, 2, 3).reshape(N, D, Sq)
    kt = jnp.swapaxes(k, 2, 3).reshape(N, D, Sk)
    vt = jnp.swapaxes(v, 2, 3).reshape(N, D, Sk)
    im = lambda i: (i, 0, 0)
    o = pl.pallas_call(
        kernel,
        grid=(N // hb,),
        in_specs=[pl.BlockSpec((hb, D, Sq), im), pl.BlockSpec((hb, D, Sk), im), pl.BlockSpec((hb, D, Sk), im)],
        out_specs=pl.BlockSpec((hb, D, Sq), im),
        out_shape=jax.ShapeDtypeStruct((N, D, Sq), q.dtype),
        compiler_params=pltpu.CompilerParams(dimension_semantics=("arbitrary",), vmem_limit_bytes=100 * 1024 * 1024),
    )(qt, kt, vt)
    return jnp.swapaxes(o.reshape(B, Hq, D, Sq), 2, 3)
```

```python
import contextlib
import math

import numpy as np
import jax
import jax.numpy as jnp
from jax import lax
import jax.experimental.pallas as pl
import jax.experimental.pallas.tpu as pltpu

B, H, Sq, Sk, D = 16, 32, 368, 512, 192
N = B * H
C = (D ** -0.5) * math.log2(math.e)
f32 = jnp.float32
bf16 = jnp.bfloat16

def col_to_row(l):
    n = l.shape[0]
    lb = jnp.broadcast_to(l, (n,128))
    diff = lax.broadcasted_iota(jnp.int32,(8,128),1) - lax.broadcasted_iota(jnp.int32,(8,128),0)
    outs = []
    for a in range(0,n,128):
        acc = jnp.zeros((8,128),f32)
        for r in range(a, min(a+128,n), 8):
            acc = jnp.where(diff == (r-a), lb[r:r+8], acc)
        outs.append(jnp.sum(acc,axis=0,keepdims=True))
    return jnp.concatenate(outs,axis=1)[:, :n]

def softmax_parts(s):
    m = jnp.max(s,axis=1,keepdims=True)
    p = jnp.exp2((s-m)*C)
    ps = [p[:,a:a+128] for a in range(0,Sk,128)]
    l4 = (ps[0]+ps[1])+(ps[2]+ps[3])
    l = col_to_row(jnp.sum(l4,axis=1,keepdims=True))
    ps[3] = jnp.minimum(ps[3], l4)
    return jnp.concatenate(ps,axis=1).astype(bf16), 1.0/l

def make(ua=4, na=11, ra=6, ga=2, um=16, nr=22, rm=20, gm=4, NK=128, qrows=48, G=35, wg=2, wrows=8,
         taper=((18,16),(2,192),(1,192),(1,192)), pkv=1, pq=0, pw=0, semchk=False, flags=None, scopes=False, smx=softmax_parts, tcap=6, w_early=0):
    scope = (lambda n: jax.named_scope(n)) if scopes else (lambda n: contextlib.nullcontext())
    bm = ua*na
    nm = (N-1-bm)//um
    ul = N - bm - nm*um
    kv0 = N - ra*na - rm*nr
    PP = D//qrows
    q0 = kv0-2
    off = (-bm) % um
    NB = 16
    assert kv0 >= ua and q0 >= ua and kv0 % ga == 0 and ra % ga == 0 and rm % gm == 0 and (kv0+ra*na+off) % gm == 0
    assert NK % um == 0 and um % gm == 0 and ua % ga == 0 and off % ga == 0
    assert N - (bm+nr*um) + gm <= NK and kv0+ra*na-2 >= bm+um
    nwb = nm-nr
    assert nwb*wg*G + sum(a for a,_ in taper) == N, (nwb*wg*G, ul)
    WP = D//wrows
    for i in range(nwb):
        for t in range(wg): assert (i*wg+t+1)*G <= bm+(nr+i)*um + (t*WP*um)//(wg*WP) + 1
    lg = lambda x: int(math.log2(x))

    def kern(zero_ref,q_hbm,k_hbm,v_hbm,o_hbm,qo,kb,vb,k0,qt_s,s_s,psem,isem,wsem):
        st = lambda x: isinstance(x,(int,np.integer))
        div = lambda c,m: c//m if st(c) else (c >> lg(m) if m & (m-1) == 0 else lax.div(c,m))
        mod = lambda c,m: c%m if st(c) else (c & (m-1) if m & (m-1) == 0 else lax.rem(c,m))
        slot = lambda g: mod(g+off,NK)
        def sem_of(g, early):
            main = mod(div(g+off,um),NB)
            if not early: return main
            if st(g): return NB + g//ua if g < bm else main
            return jnp.where(g < bm, NB + div(g,ua), main)
        def k_copy(g,n,e): return pltpu.make_async_copy(k_hbm.at[pl.ds(g+1,n)], kb.at[pl.ds(slot(g),n)], isem.at[0,sem_of(g,e)])
        def v_copy(g,n,e): return pltpu.make_async_copy(v_hbm.at[pl.ds(g,n)], vb.at[pl.ds(slot(g),n)], isem.at[1,sem_of(g,e)])
        def q_copy(g,r0,rows,e): return pltpu.make_async_copy(q_hbm.at[g+2,pl.ds(r0,rows)], qo.at[g+2,pl.ds(r0,rows)], isem.at[2,sem_of(g,e)])
        def in_wait(g,n,e):
            lim = lambda d: min(n, N-d-g) if st(g) else n
            for a,(buf,s,m) in enumerate(((kb,slot(g),lim(1)),(vb,slot(g),n),(qo,g+2,lim(2)))):
                if m > 0:
                    d = buf.at[pl.ds(s,m)]
                    pltpu.make_async_copy(d,d,isem.at[a,sem_of(g,e)]).wait()
        def w_copy(h0,n,r0,rows):
            return pltpu.make_async_copy(qo.at[pl.ds(h0,n),pl.ds(r0,rows)], o_hbm.at[pl.ds(h0,n),pl.ds(r0,rows)], wsem)

        first = [pltpu.make_async_copy(q_hbm.at[pl.ds(0,2)], qo.at[pl.ds(0,2)], psem.at[0]), pltpu.make_async_copy(k_hbm.at[0], k0, psem.at[1])]
        for c in first: c.start(priority=0)
        def init(a,b):
            for g in range(a,b,ga):
                k_copy(g,ga,True).start(priority=pkv); v_copy(g,ga,True).start(priority=pkv)
            for g in range(a,min(b,q0)): q_copy(g,0,D,True).start(priority=pkv)
        init(0,ua)
        with scope("first"):
            for c in first: c.wait()
        q_first = qo[0].T
        qt_s[...] = qo[1].T
        s_s[...] = jnp.dot(q_first, k0[...], preferred_element_type=f32)
        init(ua,kv0)

        def block(b,u,early,ops,last=False):
            with scope("wait%d"%u):
                in_wait(b,u,early)
            bo = b + zero_ref[0]
            bk = slot(b)
            qs = {1: qt_s[...]}
            def ldq(h):
                if last and h >= u: return
                if h <= u: qs[h] = qo[b+h].T
                elif h == u+1: qt_s[...] = qo[b+h].T
            ldq(2)
            s = {0: s_s[...]}
            for h in range(u):
                if not (last and h == u-1):
                    s[h+1] = jnp.dot(qs.pop(h+1), kb[bk+h], preferred_element_type=f32)
                    if h == u-1: s_s[...] = s.pop(h+1)
                p, r = smx(s.pop(h))
                o = lax.dot_general(vb[bk+h], p, (((1,),(1,)),((),())), preferred_element_type=f32)
                o = (o*r).astype(bf16)
                for ti,a in enumerate(range(0,Sq,128)):
                    qo[bo+h,:,a:min(a+128,Sq)] = o[:,a:min(a+128,Sq)]
                    ops(h,ti)
                ldq(h+3)
        NT = 3
        def share(total, u, h, ti):
            j = h*NT+ti
            return range(-(-j*total//(u*NT)), -(-(j+1)*total//(u*NT)))
        def reads(g0,rate,gr,u,e,h,ti,is_last=None):
            for j in share(rate//gr,u,h,ti):
                g = g0+j*gr
                if is_last is not None and j == rate//gr-1:
                    pl.when(jnp.logical_not(is_last))(lambda: k_copy(g,gr,e).start(priority=pkv))
                    pl.when(is_last)(lambda: k_copy(g,gr-1,e).start(priority=pkv))
                else: k_copy(g,gr,e).start(priority=pkv)
                v_copy(g,gr,e).start(priority=pkv)
            for t in share(rate*PP,u,h,ti):
                q_copy(g0-2+t//PP,(t%PP)*qrows,qrows,e).start(priority=pq)
        def body_a(i,_):
            block(i*ua,ua,True,lambda h,ti: reads(kv0+i*ra,ra,ga,ua,True,h,ti))
        lax.fori_loop(0,na,body_a,None)
        def body_m(i,_):
            def ops(h,ti):
                pl.when(i < nr)(lambda: reads(kv0+na*ra+i*rm,rm,gm,um,False,h,ti,i==nr-1))
                @pl.when(i >= nr)
                def _():
                    for w in share(wg*WP,um,h,ti):
                        w_copy(((i-nr)*wg+w//WP)*G,G,(w%WP)*wrows,wrows).start(priority=pw)
            block(bm+i*um,um,False,ops)
        lax.fori_loop(0,nm,body_m,None)
        pend = []; h0 = nwb*wg*G
        for n,rows in taper:
            pend += [(h0+n, (h0,n,r0,rows)) for r0 in range(0,D,rows)]; h0 += n
        def ops_l(h,ti):
            done = N-ul+h+(ti==NT-1); cnt = 0
            while pend and pend[0][0] <= done and (cnt < tcap or done == N):
                w_copy(*pend.pop(0)[1]).start(priority=pw); cnt += 1
        block(N-ul,ul,False,ops_l,last=True)
        assert not pend
        with scope("final"):
            pltpu.make_async_copy(qo,o_hbm,wsem).wait()
    def f(q,k,v):
        qt = jnp.swapaxes(q,2,3).reshape(N,D,Sq)
        kt = jnp.swapaxes(k,2,3).reshape(N,D,Sk)
        vt = jnp.swapaxes(v,2,3).reshape(N,D,Sk)
        o = pl.pallas_call(kern,
            in_specs=[pl.BlockSpec(memory_space=pltpu.SMEM)]+[pl.BlockSpec(memory_space=pl.ANY)]*3,
            out_specs=pl.BlockSpec(memory_space=pl.ANY),
            out_shape=jax.ShapeDtypeStruct((N,D,Sq), q.dtype),
            scratch_shapes=[pltpu.VMEM((N,D,Sq), q.dtype), pltpu.VMEM((NK,D,Sk), q.dtype), pltpu.VMEM((NK,D,Sk), q.dtype), pltpu.VMEM((D,Sk), q.dtype),
                            pltpu.VMEM((Sq,D), q.dtype), pltpu.VMEM((Sq,Sk), f32),
                            pltpu.SemaphoreType.DMA((2,)), pltpu.SemaphoreType.DMA((3,NB+na)), pltpu.SemaphoreType.DMA(())],
            compiler_params=pltpu.CompilerParams(vmem_limit_bytes=127*1024*1024, flags=flags, disable_bounds_checks=True, disable_semaphore_checks=not semchk),
        )(np.zeros((1,),np.int32),qt,kt,vt)
        return jnp.swapaxes(o.reshape(B,H,D,Sq),2,3)
    return jax.jit(f)


@jax.jit
def pallas_standalone__gqa_softmax__near_ridge_kernel(q, k, v):
    return make()(q, k, v)
```

```python
import functools
import math

import jax
import jax.numpy as jnp
from jax import lax
import jax.experimental.pallas as pl
import jax.experimental.pallas.tpu as pltpu

LANES = 128
GROUP = 4
RING = 128
STAGES = ((2, 3), (4, 4), (8, 13), (32, 12))
LAST = 2
PIECES = 3
KV_PRELOAD = 3
KV_RATE = (31, 8)
Q_PERIOD = 3
WRITE_START = 394
WRITES_PER_STEP = 3
WRITE_SHAPE = (9, 32)
WRITE_TAIL = ((20, 48), (16, 48), (4, 192), (2, 192), (1, 192), (1, 192))
SCORE_TAPS = ((0, 0), (160, 0), (320, 0), (112, 256))
V_SPLIT = (64, None, 112)


def _is_static(x):
    return isinstance(x, int)


def _div(x, m):
    if _is_static(x):
        return x // m
    return x >> (m.bit_length() - 1) if m & (m - 1) == 0 else lax.div(x, m)


def _mod(x, m):
    if _is_static(x):
        return x % m
    return x & (m - 1) if m & (m - 1) == 0 else lax.rem(x, m)


def _cdiv(a, b):
    return -(-a // b)


def _dot_nt(a, b):
    return lax.dot_general(
        a, b, (((1,), (1,)), ((), ())), preferred_element_type=jnp.float32
    )


def _softmax_tile(s, c, prev):
    rows, cols = s.shape
    m = jnp.max(s, axis=1, keepdims=True)
    p = jnp.exp2((s - m) * c)
    parts = [p[:, a : a + LANES] for a in range(0, cols, LANES)]
    half = len(parts) // 2
    acc = functools.reduce(jnp.add, parts[:half]) + functools.reduce(jnp.add, parts[half:])
    if rows < LANES:
        acc = jnp.concatenate([acc, jnp.ones((LANES - rows, LANES), acc.dtype)], axis=0)
    inv = 1.0 / jnp.sum(acc.T, axis=0, keepdims=True)
    if prev is not None:
        prev = jnp.broadcast_to(prev, (8, LANES))
        tail = jnp.where(prev < 0, prev, parts[0][rows - 8 :])
        parts[0] = jnp.concatenate([parts[0][: rows - 8], tail], axis=0)
    return jnp.concatenate(parts, axis=1).astype(jnp.bfloat16), inv


def _attention(q, k, v):
    N, D, Sk = k.shape
    Sq = q.shape[-1]
    c = D**-0.5 * math.log2(math.e)
    assert sum(u * n for u, n in STAGES) + LAST == N
    assert 2 * LANES < Sq <= 3 * LANES and LANES < D and Sk % (2 * LANES) == 0

    main, n_main = STAGES[-1]
    main_start = N - LAST - main * n_main
    shift = -main_start % main
    n_ramp = sum(n for _, n in STAGES[:-1])
    n_blocks = n_ramp + n_main + 1
    n_slots = 1 + len(SCORE_TAPS) + len(V_SPLIT)
    piece_rows = D // PIECES
    n_groups = N // GROUP

    def block_of(g, in_ramp):
        idx = n_ramp + _div(g - main_start, main)
        if in_ramp:
            end, base = main_start, n_ramp
            for u, n in reversed(STAGES[:-1]):
                start, base = end - u * n, base - n
                ramp_idx = base + _div(g - start, u)
                if _is_static(g):
                    idx = ramp_idx if g < end else idx
                else:
                    idx = jnp.where(g < end, ramp_idx, idx)
                end = start
        return idx

    def q_groups_by(g):
        return 2 + _cdiv(g, Q_PERIOD)

    def kv_per_block(u):
        return _cdiv(KV_RATE[0] * u, KV_RATE[1])

    def kv_requests(u, h, slot):
        total, j = 2 * kv_per_block(u), h * n_slots + slot
        return range(_cdiv(j * total, u * n_slots), _cdiv((j + 1) * total, u * n_slots))

    assert RING % main == 0 and main_start + shift <= RING and STAGES[0] == (2, 3)
    start, first = 0, KV_PRELOAD * PIECES
    for u, n in STAGES:
        for _ in range(n):
            assert first >= (start + u) * PIECES
            assert q_groups_by(start) * GROUP >= start + u + 2
            assert u < GROUP or (u % GROUP == 0 and (start + 2) % GROUP == 0)
            for h in range(u):
                for slot in range(n_slots):
                    for j in kv_requests(u, h, slot):
                        g = (first + j // 2) // PIECES
                        assert min(g, N - 1) < start + h + RING
                        assert u == main or g < N - 1
            start, first = start + u, first + kv_per_block(u)
    assert first >= N * PIECES and q_groups_by(main_start) < n_groups <= q_groups_by(start)

    w_groups, w_rows = WRITE_SHAPE
    w_slices = GROUP * D // w_rows
    head = N - sum(n for n, _ in WRITE_TAIL)
    n_writes = head // (w_groups * GROUP) * w_slices
    w_per_block = main * WRITES_PER_STEP
    assert head % (w_groups * GROUP) == 0 and w_per_block % w_slices == 0
    for w in range(n_writes):
        step = WRITE_START + w // WRITES_PER_STEP
        assert (w // w_slices + 1) * w_groups * GROUP <= step + 1
        assert main_start <= step < N - LAST
    tail = {}
    clock = WRITE_START + n_writes / WRITES_PER_STEP
    for n, rows in WRITE_TAIL:
        whole = n % GROUP == 0
        for r in range(0, GROUP * D if whole else D, rows):
            if whole:
                idx = (pl.ds(head // GROUP, n // GROUP), r // D, pl.ds(r % D, rows))
            else:
                idx = (head // GROUP, pl.ds(head % GROUP, n), pl.ds(r, rows))
            clock = max(clock, head + n - 1)
            tail.setdefault(min(int(clock), N - 1), []).append(idx)
            clock += (n // GROUP if whole else n) * rows / (WRITES_PER_STEP * w_groups * w_rows)
        head += n

    def kernel(q_hbm, k_hbm, v_hbm, o_hbm, qo, kv, q_next, s_next,
               first_sem, kv_sem, q_sem, o_sem):
        spare = 2 * RING

        def ring(g):
            return _mod(g + shift, RING)

        def kv_copy(is_v, g, r, rows, in_ramp):
            src = v_hbm.at[g, pl.ds(r, rows)] if is_v else k_hbm.at[g + 1, pl.ds(r, rows)]
            dst = kv.at[is_v * RING + ring(g), pl.ds(r, rows)]
            return pltpu.make_async_copy(src, dst, kv_sem.at[is_v, block_of(g, in_ramp)])

        def q_heads(ref, h, n):
            if n < GROUP:
                return ref.at[_div(h, GROUP), pl.ds(_mod(h, GROUP), n)]
            return ref.at[pl.ds(_div(h, GROUP), n // GROUP)]

        def q_copy(h, n, sem):
            return pltpu.make_async_copy(q_heads(q_hbm, h, n), q_heads(qo, h, n), sem)

        def write(idx):
            pltpu.make_async_copy(qo.at[idx], o_hbm.at[idx], o_sem).start(priority=1)

        def wait_filled(dst, sem):
            pltpu.make_async_copy(dst, dst, sem).wait()

        def block(index, b, u, request_kv, after_step, last=False):
            k0 = ring(b)
            v0 = RING + k0
            wait_filled(kv.at[pl.ds(k0, u - last)], kv_sem.at[0, index])
            wait_filled(kv.at[pl.ds(v0, u)], kv_sem.at[1, index])
            if not last:
                wait_filled(q_heads(qo, b + 2, u), q_sem.at[index])

            def head(h):
                if u < GROUP:
                    return _div(b + h, GROUP), _mod(b + h, GROUP)
                return _div(b + 2, GROUP) + (h - 2) // GROUP, (h - 2) % GROUP

            qs = {1: q_next[...]}

            def load_q(h):
                if h <= u and not last:
                    qs[h] = qo[head(h)].T
                elif h == u + 1 and not last:
                    q_next[...] = qo[head(h)].T

            load_q(2)
            scores = {0: s_next[...]}
            inv = None
            for h in range(u):
                if not (last and h == u - 1):
                    s = jnp.dot(qs.pop(h + 1), kv[k0 + h], preferred_element_type=jnp.float32)
                    request_kv(h, 0)
                    for i, (r, col) in enumerate(() if last else SCORE_TAPS):
                        tap = s[r : r + 16, col : col + LANES].astype(kv.dtype)
                        kv[spare, 16 * i : 16 * (i + 1), :LANES] = tap
                        request_kv(h, 1 + i)
                    if h == u - 1:
                        s_next[...] = s
                    else:
                        scores[h + 1] = s
                s = scores.pop(h)
                for i, (lo, split) in enumerate(zip((0, 2 * LANES, LANES), V_SPLIT)):
                    hi = min(lo + LANES, Sq)
                    p, inv = _softmax_tile(s[lo:hi], c, inv)
                    if split is None:
                        bottom = _dot_nt(kv[v0 + h, LANES:], p)
                        top = _dot_nt(p, kv[v0 + h, :LANES]).T
                        request_kv(h, 1 + len(SCORE_TAPS) + i)
                        o = jnp.concatenate([top, bottom], axis=0)
                    else:
                        v_top = kv[v0 + h, :split]
                        request_kv(h, 1 + len(SCORE_TAPS) + i)
                        o = _dot_nt(jnp.concatenate([v_top, kv[v0 + h, split:]], axis=0), p)
                    qo[(*head(h), slice(None), slice(lo, hi))] = (
                        o * inv[:, : hi - lo]
                    ).astype(qo.dtype)
                after_step(h)
                load_q(h + 3)

        first_q = q_copy(0, 2, first_sem.at[0])
        first_k = pltpu.make_async_copy(k_hbm.at[0], kv.at[spare], first_sem.at[1])
        first_q.start()
        first_k.start()

        def preload(steps):
            for g in steps:
                kv_copy(0, g, 0, D, True).start(priority=1)
                kv_copy(1, g, 0, D, True).start(priority=1)

        preload(range(2))
        q_copy(2, 2, q_sem.at[0]).start(priority=1)
        first_q.wait()
        first_k.wait()
        q0 = qo[0, 0].T
        q_next[...] = qo[0, 1].T
        s_next[...] = jnp.dot(q0, kv[spare], preferred_element_type=jnp.float32)
        preload(range(2, KV_PRELOAD))
        q_copy(4, 2, q_sem.at[1]).start(priority=1)
        q_copy(6, 2, q_sem.at[2]).start(priority=1)

        def stage(i, _, *, u, n, index, start, first):
            in_ramp = u != main
            b = start + i * u
            per_block = kv_per_block(u)
            pieces = [first + i * per_block + a for a in range(PIECES)]
            pieces = [
                (_div(t, PIECES), pl.multiple_of(_mod(t, PIECES) * piece_rows, piece_rows))
                for t in pieces
            ]
            q_group = [2 + _div(b + a, Q_PERIOD) for a in range(Q_PERIOD)]
            q_due = functools.cache(lambda a, hi: (_mod(b + a, Q_PERIOD) == 0) & (i < hi))
            below = functools.cache(lambda hi: i < hi)
            within = functools.cache(lambda lo, hi: (i >= lo) & (i < hi))
            first_group = i * (w_per_block // w_slices * w_groups)

            def request_kv(h, slot):
                for j in kv_requests(u, h, slot):
                    is_v, t = j % 2, j // 2
                    g, r = pieces[t % PIECES]

                    def go():
                        kv_copy(is_v, g + t // PIECES, r, piece_rows, in_ramp).start()

                    if in_ramp:
                        go()
                    else:
                        end = (N - 1 + is_v) * PIECES
                        pl.when(below(_cdiv(end - first - t, per_block)))(go)

            def after_step(h):
                @pl.when(q_due(h % Q_PERIOD, _cdiv((n_groups - 2) * Q_PERIOD - start - h, u)))
                def _():
                    group = q_group[h % Q_PERIOD] + h // Q_PERIOD
                    sem = q_sem.at[block_of(group * GROUP - 2, in_ramp)]
                    pltpu.make_async_copy(q_hbm.at[group], qo.at[group], sem).start(priority=1)

                if in_ramp:
                    return
                for j in range(WRITES_PER_STEP):
                    w = (start + h - WRITE_START) * WRITES_PER_STEP + j
                    row = w % w_slices * w_rows

                    @pl.when(within(_cdiv(-w, w_per_block), _cdiv(n_writes - w, w_per_block)))
                    def _():
                        groups = pl.ds(first_group + w // w_slices * w_groups, w_groups)
                        write((groups, row // D, pl.ds(row % D, w_rows)))

                for at in range(n):
                    if start + at * u + h in tail:

                        @pl.when(within(at, at + 1))
                        def _():
                            for idx in tail[start + at * u + h]:
                                write(idx)

            block(index + i, b, u, request_kv, after_step)

        index, start, first = 0, 0, KV_PRELOAD * PIECES
        for u, n in STAGES:
            body = functools.partial(stage, u=u, n=n, index=index, start=start, first=first)
            lax.fori_loop(0, n, body, None)
            index, start, first = index + n, start + u * n, first + kv_per_block(u) * n

        def write_tail(h):
            for idx in tail.get(start + h, ()):
                write(idx)

        block(index, start, LAST, lambda h, slot: None, write_tail, last=True)
        wait_filled(o_hbm, o_sem)

    return pl.pallas_call(
        kernel,
        in_specs=[pl.BlockSpec(memory_space=pl.ANY)] * 3,
        out_specs=pl.BlockSpec(memory_space=pl.ANY),
        out_shape=jax.ShapeDtypeStruct(q.shape, q.dtype),
        scratch_shapes=[
            pltpu.VMEM(q.shape, q.dtype),
            pltpu.VMEM((2 * RING + 1, D, Sk), k.dtype),
            pltpu.VMEM((Sq, D), q.dtype),
            pltpu.VMEM((Sq, Sk), jnp.float32),
            pltpu.SemaphoreType.DMA((2,)),
            pltpu.SemaphoreType.DMA((2, n_blocks)),
            pltpu.SemaphoreType.DMA((n_blocks,)),
            pltpu.SemaphoreType.DMA(()),
        ],
        compiler_params=pltpu.CompilerParams(
            vmem_limit_bytes=127 * 1024 * 1024,
            disable_bounds_checks=True,
            disable_semaphore_checks=True,
        ),
    )(q, k, v)


@jax.jit
def pallas_standalone__gqa_softmax__near_ridge_kernel(
    q: jax.Array,
    k: jax.Array,
    v: jax.Array,
):
    B, H, Sq, D = q.shape
    Sk = k.shape[2]
    assert k.shape[1] == H
    o = _attention(
        jnp.swapaxes(q, 2, 3).reshape(B * H // GROUP, GROUP, D, Sq),
        jnp.swapaxes(k, 2, 3).reshape(B * H, D, Sk),
        jnp.swapaxes(v, 2, 3).reshape(B * H, D, Sk),
    )
    return jnp.swapaxes(o.reshape(B, H, D, Sq), 2, 3)
```

```python
import functools
import math

import jax
import jax.numpy as jnp
from jax import lax
import jax.experimental.pallas as pl
import jax.experimental.pallas.tpu as pltpu

LANES = 128
GROUP = 4
RING = 128
STAGES = ((2, 3), (4, 4), (8, 13), (32, 12))
LAST = 2
PIECES = 6
KV_PRELOAD = 17
KV_RATE = (31, 8)
Q_PERIOD = 3
WRITE_START = 394
WRITES_PER_STEP = 3
WRITE_SHAPE = (9, 32)
WRITE_TAIL = ((20, 48), (16, 48), (4, 192), (2, 192), (1, 192), (1, 192))
SCORE_TAPS = ((0, 0), (160, 0), (320, 0), (112, 256))
V_SPLIT = (64, None, 112)


def _is_static(x):
    return isinstance(x, int)


def _div(x, m):
    if _is_static(x):
        return x // m
    return x >> (m.bit_length() - 1) if m & (m - 1) == 0 else lax.div(x, m)


def _mod(x, m):
    if _is_static(x):
        return x % m
    return x & (m - 1) if m & (m - 1) == 0 else lax.rem(x, m)


def _cdiv(a, b):
    return -(-a // b)


def _dot_nt(a, b):
    return lax.dot_general(
        a, b, (((1,), (1,)), ((), ())), preferred_element_type=jnp.float32
    )


def _softmax_tile(s, c, prev):
    rows, cols = s.shape
    m = jnp.max(s, axis=1, keepdims=True)
    p = jnp.exp2((s - m) * c)
    parts = [p[:, a : a + LANES] for a in range(0, cols, LANES)]
    half = len(parts) // 2
    acc = functools.reduce(jnp.add, parts[:half]) + functools.reduce(jnp.add, parts[half:])
    if rows < LANES:
        acc = jnp.concatenate([acc, jnp.ones((LANES - rows, LANES), acc.dtype)], axis=0)
    inv = 1.0 / jnp.sum(acc.T, axis=0, keepdims=True)
    if prev is not None:
        prev = jnp.broadcast_to(prev, (8, LANES))
        tail = jnp.where(prev < 0, prev, parts[0][rows - 8 :])
        parts[0] = jnp.concatenate([parts[0][: rows - 8], tail], axis=0)
    return jnp.concatenate(parts, axis=1).astype(jnp.bfloat16), inv


def _attention(q, k, v):
    N, D, Sk = k.shape
    Sq = q.shape[-1]
    c = D**-0.5 * math.log2(math.e)
    assert sum(u * n for u, n in STAGES) + LAST == N
    assert 2 * LANES < Sq <= 3 * LANES and LANES < D and Sk % (2 * LANES) == 0

    main, n_main = STAGES[-1]
    main_start = N - LAST - main * n_main
    shift = -main_start % main
    n_ramp = sum(n for _, n in STAGES[:-1])
    n_blocks = n_ramp + n_main + 1
    n_slots = 1 + len(SCORE_TAPS) + len(V_SPLIT)
    piece_rows = D // PIECES
    n_groups = N // GROUP

    def block_of(g, in_ramp):
        idx = n_ramp + _div(g - main_start, main)
        if in_ramp:
            end, base = main_start, n_ramp
            for u, n in reversed(STAGES[:-1]):
                start, base = end - u * n, base - n
                ramp_idx = base + _div(g - start, u)
                if _is_static(g):
                    idx = ramp_idx if g < end else idx
                else:
                    idx = jnp.where(g < end, ramp_idx, idx)
                end = start
        return idx

    def q_groups_by(g):
        return 2 + _cdiv(g, Q_PERIOD)

    def kv_per_block(u):
        return 2 * _cdiv(KV_RATE[0] * u, KV_RATE[1])

    def kv_requests(u, h, slot):
        total, j = kv_per_block(u), h * n_slots + slot
        pairs = range(_cdiv(j * total, u * n_slots), _cdiv((j + 1) * total, u * n_slots))
        return [(pair % 2, pair // 2 * 2 + half) for pair in pairs for half in range(2)]

    assert RING % main == 0 and main_start + shift <= RING and STAGES[0] == (2, 3)
    start, first = 0, KV_PRELOAD
    for u, n in STAGES:
        for _ in range(n):
            assert first >= (start + u) * PIECES
            assert q_groups_by(start) * GROUP >= start + u + 2
            assert u < GROUP or (u % GROUP == 0 and (start + 2) % GROUP == 0)
            for h in range(u):
                for slot in range(n_slots):
                    for _, t in kv_requests(u, h, slot):
                        g = (first + t) // PIECES
                        assert min(g, N - 1) < start + h + RING
                        assert u == main or g < N - 1
            start, first = start + u, first + kv_per_block(u)
    assert first >= N * PIECES and q_groups_by(main_start) < n_groups <= q_groups_by(start)

    w_groups, w_rows = WRITE_SHAPE
    w_slices = GROUP * D // w_rows
    head = N - sum(n for n, _ in WRITE_TAIL)
    n_writes = head // (w_groups * GROUP) * w_slices
    w_per_block = main * WRITES_PER_STEP
    assert head % (w_groups * GROUP) == 0 and w_per_block % w_slices == 0
    for w in range(n_writes):
        step = WRITE_START + w // WRITES_PER_STEP
        assert (w // w_slices + 1) * w_groups * GROUP <= step + 1
        assert main_start <= step < N - LAST
    tail = {}
    clock = WRITE_START + n_writes / WRITES_PER_STEP
    for n, rows in WRITE_TAIL:
        whole = n % GROUP == 0
        for r in range(0, GROUP * D if whole else D, rows):
            if whole:
                idx = (pl.ds(head // GROUP, n // GROUP), r // D, pl.ds(r % D, rows))
            else:
                idx = (head // GROUP, pl.ds(head % GROUP, n), pl.ds(r, rows))
            clock = max(clock, head + n - 1)
            tail.setdefault(min(int(clock), N - 1), []).append(idx)
            clock += (n // GROUP if whole else n) * rows / (WRITES_PER_STEP * w_groups * w_rows)
        head += n

    def kernel(q_hbm, k_hbm, v_hbm, o_hbm, qo, kv, q_next, s_next,
               first_sem, kv_sem, q_sem, o_sem):
        spare = 2 * RING

        def ring(g):
            return _mod(g + shift, RING)

        def kv_copy(is_v, g, r, rows, in_ramp):
            src = v_hbm.at[g, pl.ds(r, rows)] if is_v else k_hbm.at[g + 1, pl.ds(r, rows)]
            dst = kv.at[is_v * RING + ring(g), pl.ds(r, rows)]
            return pltpu.make_async_copy(src, dst, kv_sem.at[is_v, block_of(g, in_ramp)])

        def q_heads(ref, h, n):
            if n < GROUP:
                return ref.at[_div(h, GROUP), pl.ds(_mod(h, GROUP), n)]
            return ref.at[pl.ds(_div(h, GROUP), n // GROUP)]

        def q_copy(h, n, sem):
            return pltpu.make_async_copy(q_heads(q_hbm, h, n), q_heads(qo, h, n), sem)

        def write(idx):
            pltpu.make_async_copy(qo.at[idx], o_hbm.at[idx], o_sem).start(priority=1)

        def wait_filled(dst, sem):
            pltpu.make_async_copy(dst, dst, sem).wait()

        def block(index, b, u, request_kv, after_step, last=False):
            k0 = ring(b)
            v0 = RING + k0
            wait_filled(kv.at[pl.ds(k0, u - last)], kv_sem.at[0, index])
            wait_filled(kv.at[pl.ds(v0, u)], kv_sem.at[1, index])
            if not last:
                wait_filled(q_heads(qo, b + 2, u), q_sem.at[index])

            def head(h):
                if u < GROUP:
                    return _div(b + h, GROUP), _mod(b + h, GROUP)
                return _div(b + 2, GROUP) + (h - 2) // GROUP, (h - 2) % GROUP

            qs = {1: q_next[...]}

            def load_q(h):
                if h <= u and not last:
                    qs[h] = qo[head(h)].T
                elif h == u + 1 and not last:
                    q_next[...] = qo[head(h)].T

            load_q(2)
            scores = {0: s_next[...]}
            inv = None
            for h in range(u):
                if not (last and h == u - 1):
                    s = jnp.dot(qs.pop(h + 1), kv[k0 + h], preferred_element_type=jnp.float32)
                    request_kv(h, 0)
                    for i, (r, col) in enumerate(() if last else SCORE_TAPS):
                        tap = s[r : r + 16, col : col + LANES].astype(kv.dtype)
                        kv[spare, 16 * i : 16 * (i + 1), :LANES] = tap
                        request_kv(h, 1 + i)
                    if h == u - 1:
                        s_next[...] = s
                    else:
                        scores[h + 1] = s
                s = scores.pop(h)
                for i, (lo, split) in enumerate(zip((0, 2 * LANES, LANES), V_SPLIT)):
                    hi = min(lo + LANES, Sq)
                    p, inv = _softmax_tile(s[lo:hi], c, inv)
                    if split is None:
                        bottom = _dot_nt(kv[v0 + h, LANES:], p)
                        top = _dot_nt(p, kv[v0 + h, :LANES]).T
                        request_kv(h, 1 + len(SCORE_TAPS) + i)
                        o = jnp.concatenate([top, bottom], axis=0)
                    else:
                        v_top = kv[v0 + h, :split]
                        request_kv(h, 1 + len(SCORE_TAPS) + i)
                        o = _dot_nt(jnp.concatenate([v_top, kv[v0 + h, split:]], axis=0), p)
                    qo[(*head(h), slice(None), slice(lo, hi))] = (
                        o * inv[:, : hi - lo]
                    ).astype(qo.dtype)
                after_step(h)
                load_q(h + 3)

        first_q = q_copy(0, 2, first_sem.at[0])
        first_k = pltpu.make_async_copy(k_hbm.at[0], kv.at[spare], first_sem.at[1])
        first_q.start()
        first_k.start()

        def preload(steps):
            for g in steps:
                rows = min(D, (KV_PRELOAD - g * PIECES) * piece_rows)
                kv_copy(0, g, 0, rows, True).start(priority=1)
                kv_copy(1, g, 0, rows, True).start(priority=1)

        preload(range(2))
        q_copy(2, 2, q_sem.at[0]).start(priority=1)
        first_q.wait()
        first_k.wait()
        q0 = qo[0, 0].T
        q_next[...] = qo[0, 1].T
        s_next[...] = jnp.dot(q0, kv[spare], preferred_element_type=jnp.float32)
        preload(range(2, _cdiv(KV_PRELOAD, PIECES)))
        q_copy(4, 2, q_sem.at[1]).start(priority=1)
        q_copy(6, 2, q_sem.at[2]).start(priority=1)

        def stage(i, _, *, u, n, index, start, first):
            in_ramp = u != main
            b = start + i * u
            per_block = kv_per_block(u)
            pieces = [first + i * per_block + a for a in range(PIECES)]
            pieces = [
                (_div(t, PIECES), pl.multiple_of(_mod(t, PIECES) * piece_rows, piece_rows))
                for t in pieces
            ]
            q_group = [2 + _div(b + a, Q_PERIOD) for a in range(Q_PERIOD)]
            q_due = functools.cache(lambda a, hi: (_mod(b + a, Q_PERIOD) == 0) & (i < hi))
            below = functools.cache(lambda hi: i < hi)
            within = functools.cache(lambda lo, hi: (i >= lo) & (i < hi))
            first_group = i * (w_per_block // w_slices * w_groups)

            def request_kv(h, slot):
                for is_v, t in kv_requests(u, h, slot):
                    g, r = pieces[t % PIECES]

                    def go():
                        kv_copy(is_v, g + t // PIECES, r, piece_rows, in_ramp).start()

                    if in_ramp:
                        go()
                    else:
                        end = (N - 1 + is_v) * PIECES
                        pl.when(below(_cdiv(end - first - t, per_block)))(go)

            def after_step(h):
                @pl.when(q_due(h % Q_PERIOD, _cdiv((n_groups - 2) * Q_PERIOD - start - h, u)))
                def _():
                    group = q_group[h % Q_PERIOD] + h // Q_PERIOD
                    sem = q_sem.at[block_of(group * GROUP - 2, in_ramp)]
                    pltpu.make_async_copy(q_hbm.at[group], qo.at[group], sem).start(priority=1)

                if in_ramp:
                    return
                for j in range(WRITES_PER_STEP):
                    w = (start + h - WRITE_START) * WRITES_PER_STEP + j
                    row = w % w_slices * w_rows

                    @pl.when(within(_cdiv(-w, w_per_block), _cdiv(n_writes - w, w_per_block)))
                    def _():
                        groups = pl.ds(first_group + w // w_slices * w_groups, w_groups)
                        write((groups, row // D, pl.ds(row % D, w_rows)))

                for at in range(n):
                    if start + at * u + h in tail:

                        @pl.when(within(at, at + 1))
                        def _():
                            for idx in tail[start + at * u + h]:
                                write(idx)

            block(index + i, b, u, request_kv, after_step)

        index, start, first = 0, 0, KV_PRELOAD
        for u, n in STAGES:
            body = functools.partial(stage, u=u, n=n, index=index, start=start, first=first)
            lax.fori_loop(0, n, body, None)
            index, start, first = index + n, start + u * n, first + kv_per_block(u) * n

        def write_tail(h):
            for idx in tail.get(start + h, ()):
                write(idx)

        block(index, start, LAST, lambda h, slot: None, write_tail, last=True)
        wait_filled(o_hbm, o_sem)

    return pl.pallas_call(
        kernel,
        in_specs=[pl.BlockSpec(memory_space=pl.ANY)] * 3,
        out_specs=pl.BlockSpec(memory_space=pl.ANY),
        out_shape=jax.ShapeDtypeStruct(q.shape, q.dtype),
        scratch_shapes=[
            pltpu.VMEM(q.shape, q.dtype),
            pltpu.VMEM((2 * RING + 1, D, Sk), k.dtype),
            pltpu.VMEM((Sq, D), q.dtype),
            pltpu.VMEM((Sq, Sk), jnp.float32),
            pltpu.SemaphoreType.DMA((2,)),
            pltpu.SemaphoreType.DMA((2, n_blocks)),
            pltpu.SemaphoreType.DMA((n_blocks,)),
            pltpu.SemaphoreType.DMA(()),
        ],
        compiler_params=pltpu.CompilerParams(
            vmem_limit_bytes=127 * 1024 * 1024,
            disable_bounds_checks=True,
            disable_semaphore_checks=True,
        ),
    )(q, k, v)


@jax.jit
def pallas_standalone__gqa_softmax__near_ridge_kernel(
    q: jax.Array,
    k: jax.Array,
    v: jax.Array,
):
    B, H, Sq, D = q.shape
    Sk = k.shape[2]
    assert k.shape[1] == H
    o = _attention(
        jnp.swapaxes(q, 2, 3).reshape(B * H // GROUP, GROUP, D, Sq),
        jnp.swapaxes(k, 2, 3).reshape(B * H, D, Sk),
        jnp.swapaxes(v, 2, 3).reshape(B * H, D, Sk),
    )
    return jnp.swapaxes(o.reshape(B, H, D, Sq), 2, 3)
```

```python
import functools
import math

import jax
import jax.numpy as jnp
from jax import lax
import jax.experimental.pallas as pl
import jax.experimental.pallas.tpu as pltpu

LANES = 128
GROUP = 4
RING = 128
STAGES = ((2, 3), (4, 4), (8, 13), (32, 12))
LAST = 2
PIECES = 6
KV_PRELOAD = 15
KV_RATE = (31, 8)
Q_PERIOD = 3
WRITE_START = 393
WRITES_PER_STEP = 3
WRITE_SHAPE = (9, 32)
WRITE_TAIL = ((20, 48), (16, 48), (4, 192), (2, 192), (1, 192), (1, 192))
SCORE_TAPS = ((0, 0), (160, 0), (320, 0), (112, 256))
V_SPLIT = (64, None, 112)


def _is_static(x):
    return isinstance(x, int)


def _div(x, m):
    if _is_static(x):
        return x // m
    if m & (m - 1) == 0:
        return x >> (m.bit_length() - 1)
    return (x * _cdiv(1 << 16, m)) >> 16


def _mod(x, m):
    if _is_static(x):
        return x % m
    return x & (m - 1) if m & (m - 1) == 0 else x - m * _div(x, m)


def _cdiv(a, b):
    return -(-a // b)


def _dot_nt(a, b):
    return lax.dot_general(
        a, b, (((1,), (1,)), ((), ())), preferred_element_type=jnp.float32
    )


def _softmax_tile(s, c, prev):
    rows, cols = s.shape
    m = jnp.max(s, axis=1, keepdims=True)
    p = jnp.exp2((s - m) * c)
    parts = [p[:, a : a + LANES] for a in range(0, cols, LANES)]
    half = len(parts) // 2
    acc = functools.reduce(jnp.add, parts[:half]) + functools.reduce(jnp.add, parts[half:])
    if rows < LANES:
        acc = jnp.concatenate([acc, jnp.ones((LANES - rows, LANES), acc.dtype)], axis=0)
    inv = 1.0 / jnp.sum(acc.T, axis=0, keepdims=True)
    if prev is not None:
        prev = jnp.broadcast_to(prev, (8, LANES))
        tail = jnp.where(prev < 0, prev, parts[0][rows - 8 :])
        parts[0] = jnp.concatenate([parts[0][: rows - 8], tail], axis=0)
    return jnp.concatenate(parts, axis=1).astype(jnp.bfloat16), inv


def _attention(q, k, v):
    N, D, Sk = k.shape
    Sq = q.shape[-1]
    c = D**-0.5 * math.log2(math.e)
    assert sum(u * n for u, n in STAGES) + LAST == N
    assert 2 * LANES < Sq <= 3 * LANES and LANES < D and Sk % (2 * LANES) == 0

    main, n_main = STAGES[-1]
    main_start = N - LAST - main * n_main
    shift = -main_start % main
    n_ramp = sum(n for _, n in STAGES[:-1])
    n_blocks = n_ramp + n_main + 1
    n_slots = 1 + len(SCORE_TAPS) + len(V_SPLIT)
    piece_rows = D // PIECES
    n_groups = N // GROUP

    def block_of(g, in_ramp):
        idx = n_ramp + _div(g - main_start, main)
        if in_ramp:
            end, base = main_start, n_ramp
            for u, n in reversed(STAGES[:-1]):
                start, base = end - u * n, base - n
                ramp_idx = base + _div(g - start, u)
                if _is_static(g):
                    idx = ramp_idx if g < end else idx
                else:
                    idx = jnp.where(g < end, ramp_idx, idx)
                end = start
        return idx

    def q_groups_by(g):
        return 2 + _cdiv(g, Q_PERIOD)

    def kv_per_block(u):
        return 2 * _cdiv(KV_RATE[0] * u, KV_RATE[1])

    def kv_requests(u, h, slot):
        total, j = kv_per_block(u), h * n_slots + slot
        pairs = range(_cdiv(j * total, u * n_slots), _cdiv((j + 1) * total, u * n_slots))
        return [(pair % 2, pair // 2 * 2 + half) for pair in pairs for half in range(2)]

    assert RING % main == 0 and main_start + shift <= RING and STAGES[0] == (2, 3)
    start, first = 0, KV_PRELOAD
    for u, n in STAGES:
        for _ in range(n):
            assert first >= (start + u) * PIECES
            assert q_groups_by(start) * GROUP >= start + u + 2
            assert u < GROUP or (u % GROUP == 0 and (start + 2) % GROUP == 0)
            for h in range(u):
                for slot in range(n_slots):
                    for _, t in kv_requests(u, h, slot):
                        g = (first + t) // PIECES
                        assert min(g, N - 1) < start + h + RING
                        assert u == main or g < N - 1
            start, first = start + u, first + kv_per_block(u)
    assert N * PIECES <= first < (1 << 16) // PIECES
    assert q_groups_by(main_start) < n_groups <= q_groups_by(start)

    w_groups, w_rows = WRITE_SHAPE
    w_slices = GROUP * D // w_rows
    head = N - sum(n for n, _ in WRITE_TAIL)
    n_writes = head // (w_groups * GROUP) * w_slices
    w_per_block = main * WRITES_PER_STEP
    assert head % (w_groups * GROUP) == 0 and w_per_block % w_slices == 0
    for w in range(n_writes):
        step = WRITE_START + w // WRITES_PER_STEP
        assert (w // w_slices + 1) * w_groups * GROUP <= step + 1
        assert main_start <= step < N - LAST
    tail = {}
    clock = WRITE_START + n_writes / WRITES_PER_STEP
    for n, rows in WRITE_TAIL:
        whole = n % GROUP == 0
        for r in range(0, GROUP * D if whole else D, rows):
            if whole:
                idx = (pl.ds(head // GROUP, n // GROUP), r // D, pl.ds(r % D, rows))
            else:
                idx = (head // GROUP, pl.ds(head % GROUP, n), pl.ds(r, rows))
            clock = max(clock, head + n - 1)
            tail.setdefault(min(int(clock), N - 1), []).append(idx)
            clock += (n // GROUP if whole else n) * rows / (WRITES_PER_STEP * w_groups * w_rows)
        head += n

    def kernel(q_hbm, k_hbm, v_hbm, o_hbm, qo, kv, q_next, s_next,
               first_sem, kv_sem, q_sem, o_sem):
        spare = 2 * RING

        def ring(g):
            return _mod(g + shift, RING)

        def kv_copy(is_v, g, r, rows, in_ramp):
            src = v_hbm.at[g, pl.ds(r, rows)] if is_v else k_hbm.at[g + 1, pl.ds(r, rows)]
            dst = kv.at[is_v * RING + ring(g), pl.ds(r, rows)]
            return pltpu.make_async_copy(src, dst, kv_sem.at[is_v, block_of(g, in_ramp)])

        def q_heads(ref, h, n):
            if n < GROUP:
                return ref.at[_div(h, GROUP), pl.ds(_mod(h, GROUP), n)]
            return ref.at[pl.ds(_div(h, GROUP), n // GROUP)]

        def q_copy(h, n, sem):
            return pltpu.make_async_copy(q_heads(q_hbm, h, n), q_heads(qo, h, n), sem)

        def write(idx):
            pltpu.make_async_copy(qo.at[idx], o_hbm.at[idx], o_sem).start(priority=1)

        def wait_filled(dst, sem):
            pltpu.make_async_copy(dst, dst, sem).wait()

        def wait_inputs(index, b, u, last=False):
            wait_filled(kv.at[pl.ds(ring(b), u - last)], kv_sem.at[0, index])
            wait_filled(kv.at[pl.ds(RING + ring(b), u)], kv_sem.at[1, index])
            if not last:
                wait_filled(q_heads(qo, b + 2, u), q_sem.at[index])

        def block(b, u, request_kv, after_step, last=False):
            k0 = ring(b)
            v0 = RING + k0

            def head(h):
                if u < GROUP:
                    return _div(b + h, GROUP), _mod(b + h, GROUP)
                return _div(b + 2, GROUP) + (h - 2) // GROUP, (h - 2) % GROUP

            qs = {1: q_next[...]}

            def load_q(h):
                if h <= u and not last:
                    qs[h] = qo[head(h)].T
                elif h == u + 1 and not last:
                    q_next[...] = qo[head(h)].T

            load_q(2)
            scores = {0: s_next[...]}
            inv = None
            for h in range(u):
                if not (last and h == u - 1):
                    s = jnp.dot(qs.pop(h + 1), kv[k0 + h], preferred_element_type=jnp.float32)
                    request_kv(h, 0)
                    for i, (r, col) in enumerate(() if last else SCORE_TAPS):
                        tap = s[r : r + 16, col : col + LANES].astype(kv.dtype)
                        kv[spare, 16 * i : 16 * (i + 1), :LANES] = tap
                        request_kv(h, 1 + i)
                    if h == u - 1:
                        s_next[...] = s
                    else:
                        scores[h + 1] = s
                s = scores.pop(h)
                for i, (lo, split) in enumerate(zip((0, 2 * LANES, LANES), V_SPLIT)):
                    hi = min(lo + LANES, Sq)
                    p, inv = _softmax_tile(s[lo:hi], c, inv)
                    if split is None:
                        bottom = _dot_nt(kv[v0 + h, LANES:], p)
                        top = _dot_nt(p, kv[v0 + h, :LANES]).T
                        request_kv(h, 1 + len(SCORE_TAPS) + i)
                        o = jnp.concatenate([top, bottom], axis=0)
                    else:
                        v_top = kv[v0 + h, :split]
                        request_kv(h, 1 + len(SCORE_TAPS) + i)
                        o = _dot_nt(jnp.concatenate([v_top, kv[v0 + h, split:]], axis=0), p)
                    qo[(*head(h), slice(None), slice(lo, hi))] = (
                        o * inv[:, : hi - lo]
                    ).astype(qo.dtype)
                after_step(h)
                load_q(h + 3)

        first_q = q_copy(0, 2, first_sem.at[0])
        first_k = pltpu.make_async_copy(k_hbm.at[0], kv.at[spare], first_sem.at[1])
        first_q.start()
        first_k.start()

        def preload(steps):
            for g in steps:
                rows = min(D, (KV_PRELOAD - g * PIECES) * piece_rows)
                kv_copy(0, g, 0, rows, True).start(priority=1)
                kv_copy(1, g, 0, rows, True).start(priority=1)

        preload(range(2))
        q_copy(2, 2, q_sem.at[0]).start(priority=1)
        first_q.wait()
        first_k.wait()
        q0 = qo[0, 0].T
        q_next[...] = qo[0, 1].T
        s_next[...] = jnp.dot(q0, kv[spare], preferred_element_type=jnp.float32)
        preload(range(2, _cdiv(KV_PRELOAD, PIECES)))
        q_copy(4, 2, q_sem.at[1]).start(priority=1)
        q_copy(6, 2, q_sem.at[2]).start(priority=1)

        def stage(i, _, *, u, n, index, start, first):
            in_ramp = u != main
            b = start + i * u
            first_group = i * (w_per_block // w_slices * w_groups)
            q_group = [2 + _div(b + a, Q_PERIOD) for a in range(Q_PERIOD)]
            wait_inputs(index + i, b, u)
            per_block = kv_per_block(u)
            pieces = [first + i * per_block + a for a in range(PIECES)]
            pieces = [
                (_div(t, PIECES), pl.multiple_of(_mod(t, PIECES) * piece_rows, piece_rows))
                for t in pieces
            ]
            q_due = functools.cache(lambda a, hi: (_mod(b + a, Q_PERIOD) == 0) & (i < hi))
            below = functools.cache(lambda hi: i < hi)
            within = functools.cache(lambda lo, hi: (i >= lo) & (i < hi))

            def request_kv(h, slot):
                for is_v, t in kv_requests(u, h, slot):
                    g, r = pieces[t % PIECES]

                    def go():
                        kv_copy(is_v, g + t // PIECES, r, piece_rows, in_ramp).start()

                    if in_ramp:
                        go()
                    else:
                        end = (N - 1 + is_v) * PIECES
                        pl.when(below(_cdiv(end - first - t, per_block)))(go)

            def after_step(h):
                @pl.when(q_due(h % Q_PERIOD, _cdiv((n_groups - 2) * Q_PERIOD - start - h, u)))
                def _():
                    group = q_group[h % Q_PERIOD] + h // Q_PERIOD
                    sem = q_sem.at[block_of(group * GROUP - 2, in_ramp)]
                    pltpu.make_async_copy(q_hbm.at[group], qo.at[group], sem).start(priority=1)

                if in_ramp:
                    return
                for j in range(WRITES_PER_STEP):
                    w = (start + h - WRITE_START) * WRITES_PER_STEP + j
                    row = w % w_slices * w_rows

                    @pl.when(within(_cdiv(-w, w_per_block), _cdiv(n_writes - w, w_per_block)))
                    def _():
                        groups = pl.ds(first_group + w // w_slices * w_groups, w_groups)
                        write((groups, row // D, pl.ds(row % D, w_rows)))

                for at in range(n):
                    if start + at * u + h in tail:

                        @pl.when(within(at, at + 1))
                        def _():
                            for idx in tail[start + at * u + h]:
                                write(idx)

            block(b, u, request_kv, after_step)

        index, start, first = 0, 0, KV_PRELOAD
        for u, n in STAGES:
            body = functools.partial(stage, u=u, n=n, index=index, start=start, first=first)
            lax.fori_loop(0, n, body, None)
            index, start, first = index + n, start + u * n, first + kv_per_block(u) * n

        def write_tail(h):
            for idx in tail.get(start + h, ()):
                write(idx)

        wait_inputs(index, start, LAST, last=True)
        block(start, LAST, lambda h, slot: None, write_tail, last=True)
        wait_filled(o_hbm, o_sem)

    return pl.pallas_call(
        kernel,
        in_specs=[pl.BlockSpec(memory_space=pl.ANY)] * 3,
        out_specs=pl.BlockSpec(memory_space=pl.ANY),
        out_shape=jax.ShapeDtypeStruct(q.shape, q.dtype),
        scratch_shapes=[
            pltpu.VMEM(q.shape, q.dtype),
            pltpu.VMEM((2 * RING + 1, D, Sk), k.dtype),
            pltpu.VMEM((Sq, D), q.dtype),
            pltpu.VMEM((Sq, Sk), jnp.float32),
            pltpu.SemaphoreType.DMA((2,)),
            pltpu.SemaphoreType.DMA((2, n_blocks)),
            pltpu.SemaphoreType.DMA((n_blocks,)),
            pltpu.SemaphoreType.DMA(()),
        ],
        compiler_params=pltpu.CompilerParams(
            vmem_limit_bytes=127 * 1024 * 1024,
            disable_bounds_checks=True,
            disable_semaphore_checks=True,
        ),
    )(q, k, v)


@jax.jit
def pallas_standalone__gqa_softmax__near_ridge_kernel(
    q: jax.Array,
    k: jax.Array,
    v: jax.Array,
):
    B, H, Sq, D = q.shape
    Sk = k.shape[2]
    assert k.shape[1] == H
    o = _attention(
        jnp.swapaxes(q, 2, 3).reshape(B * H // GROUP, GROUP, D, Sq),
        jnp.swapaxes(k, 2, 3).reshape(B * H, D, Sk),
        jnp.swapaxes(v, 2, 3).reshape(B * H, D, Sk),
    )
    return jnp.swapaxes(o.reshape(B, H, D, Sq), 2, 3)
```
